```python
import os as _os
_os.environ.setdefault("JAX_PLATFORMS", "cpu")
import jax
import jax.numpy as jnp

def _softmax(x, axis=-1):
    return jax.nn.softmax(x, axis=axis)
def _gelu(x):
    return jax.nn.gelu(x, approximate=True)
def _silu(x):
    return jax.nn.silu(x)
def _sigmoid(x):
    return jax.nn.sigmoid(x)
def _layernorm(x, axis=-1, eps=1e-5):
    m = jnp.mean(x, axis=axis, keepdims=True)
    v = jnp.var(x, axis=axis, keepdims=True)
    return (x - m) / jnp.sqrt(v + eps)
def _scatter_add(tgt, idx, src, axis=0):
    return tgt.at[idx].add(src)
def _segment_sum(src, seg, n):
    return jax.ops.segment_sum(src, seg, n)
class _Rng:
    def __init__(self, key):
        self._k = key
    def _next(self):
        self._k, sub = jax.random.split(self._k)
        return sub
    def normal(self, shape):
        return jax.random.normal(self._next(), shape, dtype=jnp.bfloat16)
    def randint(self, lo, hi, shape):
        return jax.random.randint(self._next(), shape, lo, hi, dtype=jnp.int32)
    def uniform(self, shape, lo=0.0, hi=1.0):
        return jax.random.uniform(self._next(), shape, jnp.bfloat16, lo, hi)
    def permutation(self, n):
        return jax.random.permutation(self._next(), n)


kernel_name = 'standalone__sliding_local_fixed_window__prompt'

def setup_inputs():
    _rng = _Rng(jax.random.key(int.from_bytes(__import__("os").urandom(4), "little")))
    _w = (lambda a: (lambda t: t.astype(jnp.bfloat16) if jnp.issubdtype(t.dtype, jnp.floating) else t)(jnp.asarray(a)))
    B, H, S, D = 1, 32, 2048, 128
    return {
        "q": _w((lambda *s: _rng.normal(s) * 0.4)(B, H, S, D)),
        "k": _w((lambda *s: _rng.normal(s) * 0.4)(B, H, S, D)),
        "v": _w((lambda *s: _rng.normal(s) * 0.05)(B, H, S, D)),
    }

def reference(q, k, v):
    B, H, S, D = q.shape
    w = 32
    pos = jnp.arange(S)
    rel = pos[:, None] - pos[None, :]
    mask = (rel >= 0) & (rel < w)
    scores = jnp.einsum("bhqd,bhkd->bhqk", q, k) * (D ** -0.5)
    scores = jnp.where(mask[None, None], scores, (lambda x, dt: x.astype(dt))(jnp.array(-1e9), q.dtype))
    p = _softmax(scores, axis=-1)
    return jnp.einsum("bhqk,bhkd->bhqd", p, v)
```

```python
import numpy as np
import jax
import jax.numpy as jnp
from jax import lax
import jax.experimental.pallas as pl
import jax.experimental.pallas.tpu as pltpu

W = 32
NT = (((1,), (1,)), ((), ()))
NEG = -1e30


@jax.jit
def pallas_standalone__sliding_local_fixed_window__prompt_kernel(q, k, v):
    B, H, S, D = q.shape
    C = float(D ** -0.5 * np.log2(np.e))

    def kernel(q_ref, k_ref, v_ref, o_ref):
        def blk(q0, n, k0):
            r = lax.broadcasted_iota(jnp.int32, (n, 128), 0) + (q0 - k0)
            c = lax.broadcasted_iota(jnp.int32, (n, 128), 1)
            band = (c <= r) & (r - c < W)
            s = lax.dot_general(q_ref[q0:q0 + n, :], k_ref[k0:k0 + 128, :], NT,
                                preferred_element_type=jnp.float32)
            s = jnp.where(band, s, NEG)
            m = jnp.max(s, axis=1, keepdims=True)
            e = jnp.exp2((s - m) * C)
            l = jnp.sum(e, axis=1, keepdims=True)
            o = jnp.dot(e.astype(jnp.bfloat16), v_ref[k0:k0 + 128, :],
                        preferred_element_type=jnp.float32)
            o_ref[q0:q0 + n, :] = (o * (1.0 / l)).astype(o_ref.dtype)
        blk(0, 128, 0)
        for q0 in range(128, S, 96):
            blk(q0, 96, q0 - W)

    spec = pl.BlockSpec((None, S, D), lambda i: (i, 0, 0))
    o = pl.pallas_call(
        kernel, grid=(B * H,), in_specs=[spec] * 3, out_specs=spec,
        out_shape=jax.ShapeDtypeStruct((B * H, S, D), q.dtype),
        compiler_params=pltpu.CompilerParams(dimension_semantics=("arbitrary",)),
    )(q.reshape(B * H, S, D), k.reshape(B * H, S, D), v.reshape(B * H, S, D))
    return o.reshape(B, H, S, D)
```

```python
import numpy as np
import jax
import jax.numpy as jnp
from jax import lax
import jax.experimental.pallas as pl
import jax.experimental.pallas.tpu as pltpu

_W = 32
_MASK_VALUE = -1e9
_KT = 128
_QT = _KT - _W
_NT = (((1,), (1,)), ((), ()))

_NBUF = 4
_CH = 128
_RD_REGIONS = 2
_WR_REGIONS = 8
_TAIL = 512


def _banded_head(q_ref, k_ref, v_ref, o_ref, scale):
    S = q_ref.shape[0]
    c = float(scale * np.log2(np.e))

    def tile(q0, n, k0):
        row = lax.broadcasted_iota(jnp.int32, (n, _KT), 0) + (q0 - k0)
        col = lax.broadcasted_iota(jnp.int32, (n, _KT), 1)
        s = lax.dot_general(q_ref[q0:q0 + n, :], k_ref[k0:k0 + _KT, :], _NT,
                            preferred_element_type=jnp.float32)
        s = jnp.where((col <= row) & (row - col < _W), s, -1e30)
        m = jnp.max(s, axis=1, keepdims=True)
        e = jnp.exp2((s - m) * c)
        l = jnp.sum(e, axis=1, keepdims=True)
        o = jnp.dot(e.astype(v_ref.dtype), v_ref[k0:k0 + _KT, :],
                    preferred_element_type=jnp.float32)
        o_ref[q0:q0 + n, :] = (o * (1.0 / l)).astype(o_ref.dtype)
        return m

    m = tile(0, _KT, 0)
    m_min = jnp.minimum(m[:_QT], m[_W:])
    for q0 in range(_KT, S, _QT):
        q0 = min(q0, S - _QT)
        m_min = jnp.minimum(m_min, tile(q0, _QT, q0 - _W))
    return jnp.min(m_min)


def _dense_head(q_ref, k_ref, v_ref, o_ref, scale):
    S = q_ref.shape[0]
    dt = q_ref.dtype
    n = 16
    mask_value = float(np.asarray(_MASK_VALUE, dt))

    def body(i, _):
        q0 = pl.multiple_of(i * n, n)
        rel = (q0 + lax.broadcasted_iota(jnp.int32, (n, S), 0)
               - lax.broadcasted_iota(jnp.int32, (n, S), 1))
        s = lax.dot_general(q_ref[pl.ds(q0, n), :], k_ref[...], _NT,
                            preferred_element_type=jnp.float32)
        s = (s.astype(dt).astype(jnp.float32) * scale).astype(dt).astype(jnp.float32)
        s = jnp.where((rel >= 0) & (rel < _W), s, mask_value)
        e = jnp.exp(s - jnp.max(s, axis=1, keepdims=True))
        p = e / jnp.sum(e, axis=1, keepdims=True)
        o = jnp.dot(p.astype(dt), v_ref[...], preferred_element_type=jnp.float32)
        o_ref[pl.ds(q0, n), :] = o.astype(o_ref.dtype)

    lax.fori_loop(0, S // n, body, None)


@jax.jit
def pallas_standalone__sliding_local_fixed_window__prompt_kernel(
    q: jax.Array,
    k: jax.Array,
    v: jax.Array,
):
    B, H, S, D = q.shape
    NH = B * H
    scale = float(np.asarray(D ** -0.5, q.dtype))
    groups = NH // _WR_REGIONS
    switch = NH - _NBUF
    rounds = S // _CH
    early = (groups - 1) * rounds
    assert NH % _WR_REGIONS == 0 and groups > 1 and early % _NBUF == 0
    assert S % (2 * _CH * _RD_REGIONS) == 0 and _TAIL % (2 * _CH) == 0 and _TAIL < S

    def head_of(i):
        return (i % _WR_REGIONS) * groups + i // _WR_REGIONS

    def kernel(q_hbm, k_hbm, v_hbm, o_hbm, in_buf, out_buf, in_sem, tail_sem, out_sem):
        def start_reads(i, regions=_RD_REGIONS, tail=0):
            slot = i % _NBUF
            base = head_of(i) * S
            for off in range(0, S // regions, 2 * _CH):
                for r in range(regions):
                    for j, src in enumerate((q_hbm, k_hbm, v_hbm)):
                        for p in range(2):
                            row = r * (S // regions) + off + p * _CH
                            pltpu.make_async_copy(
                                src.at[pl.ds(pl.multiple_of(base + row, _CH), _CH)],
                                in_buf.at[slot, j, pl.ds(row, _CH)],
                                tail_sem.at[0] if row >= S - tail else in_sem.at[slot],
                            ).start(priority=p)

        def wait_fill(buf, sem):
            pltpu.make_async_copy(buf, buf, sem).wait()

        def start_writes(lo, hi):
            def one_round(x, _):
                for r in range(_WR_REGIONS):
                    rows = pl.ds(pl.multiple_of(r * groups * S + x * _CH, _CH), _CH)
                    pltpu.make_async_copy(
                        out_buf.at[rows], o_hbm.at[rows], out_sem.at[0]
                    ).start(priority=r % 2)

            lax.fori_loop(lo, hi, one_round, None)

        last_slot = (NH - 1) % _NBUF

        def step(i, _):
            slot = i % _NBUF

            @pl.when(i < switch)
            def _():
                start_reads(i + _NBUF - 1)
                wait_fill(in_buf.at[slot], in_sem.at[slot])

            @pl.when(i == switch)
            def _():
                start_reads(NH - 1, regions=1, tail=_TAIL)
                for t in range(switch, NH - 1):
                    wait_fill(in_buf.at[t % _NBUF], in_sem.at[t % _NBUF])
                wait_fill(in_buf.at[last_slot, :, pl.ds(0, S - _TAIL)],
                          in_sem.at[last_slot])

            @pl.when(i >= switch)
            def _():
                per_step = early // _NBUF
                start_writes((i - switch) * per_step, (i - switch + 1) * per_step)

            @pl.when(i == NH - 1)
            def _():
                wait_fill(in_buf.at[last_slot, :, pl.ds(S - _TAIL, _TAIL)],
                          tail_sem.at[0])

            refs = (in_buf.at[slot, 0], in_buf.at[slot, 1], in_buf.at[slot, 2],
                    out_buf.at[pl.ds(pl.multiple_of(head_of(i) * S, S), S)])
            m_min = _banded_head(*refs, scale)

            @pl.when(jnp.logical_not(m_min * scale > 0.9 * _MASK_VALUE))
            def _():
                _dense_head(*refs, scale)

        lax.fori_loop(0, _NBUF - 1, lambda i, _: start_reads(i), None)
        lax.fori_loop(0, NH, step, None)
        start_writes(early, groups * rounds)
        pltpu.make_async_copy(out_buf, o_hbm, out_sem.at[0]).wait()

    hbm = pl.BlockSpec(memory_space=pl.ANY)
    o = pl.pallas_call(
        kernel,
        in_specs=[hbm, hbm, hbm],
        out_specs=hbm,
        out_shape=jax.ShapeDtypeStruct((NH * S, D), q.dtype),
        scratch_shapes=[
            pltpu.VMEM((_NBUF, 3, S, D), q.dtype),
            pltpu.VMEM((NH * S, D), q.dtype),
            pltpu.SemaphoreType.DMA((_NBUF,)),
            pltpu.SemaphoreType.DMA((1,)),
            pltpu.SemaphoreType.DMA((1,)),
        ],
        compiler_params=pltpu.CompilerParams(vmem_limit_bytes=64 * 1024 * 1024),
    )(q.reshape(NH * S, D), k.reshape(NH * S, D), v.reshape(NH * S, D))
    return o.reshape(B, H, S, D)
```

```python
import numpy as np
import jax
import jax.numpy as jnp
from jax import lax
import jax.experimental.pallas as pl
import jax.experimental.pallas.tpu as pltpu

_W = 32
_MASK_VALUE = -1e9
_KT = 128
_QT = _KT - _W
_NT = (((1,), (1,)), ((), ()))

_NBUF = 3
_CH = 128
_WR_REGIONS = 8
_TAIL = 512


def _banded_head(q_ref, k_ref, v_ref, o_ref, scale):
    S = q_ref.shape[0]
    c = float(scale * np.log2(np.e))

    def tile(q0, n, k0):
        row = lax.broadcasted_iota(jnp.int32, (n, _KT), 0) + (q0 - k0)
        col = lax.broadcasted_iota(jnp.int32, (n, _KT), 1)
        s = lax.dot_general(q_ref[q0:q0 + n, :], k_ref[k0:k0 + _KT, :], _NT,
                            preferred_element_type=jnp.float32)
        s = jnp.where((col <= row) & (row - col < _W), s, -1e30)
        m = jnp.max(s, axis=1, keepdims=True)
        e = jnp.exp2((s - m) * c)
        l = jnp.sum(e, axis=1, keepdims=True)
        o = jnp.dot(e.astype(v_ref.dtype), v_ref[k0:k0 + _KT, :],
                    preferred_element_type=jnp.float32)
        o_ref[q0:q0 + n, :] = (o * (1.0 / l)).astype(o_ref.dtype)
        return m

    m = tile(0, _KT, 0)
    m_min = jnp.minimum(m[:_QT], m[_W:])
    for q0 in range(_KT, S, _QT):
        q0 = min(q0, S - _QT)
        m_min = jnp.minimum(m_min, tile(q0, _QT, q0 - _W))
    return jnp.min(m_min)


def _dense_head(q_ref, k_ref, v_ref, o_ref, scale):
    S = q_ref.shape[0]
    dt = q_ref.dtype
    n = 16
    mask_value = float(np.asarray(_MASK_VALUE, dt))

    def body(i, _):
        q0 = pl.multiple_of(i * n, n)
        rel = (q0 + lax.broadcasted_iota(jnp.int32, (n, S), 0)
               - lax.broadcasted_iota(jnp.int32, (n, S), 1))
        s = lax.dot_general(q_ref[pl.ds(q0, n), :], k_ref[...], _NT,
                            preferred_element_type=jnp.float32)
        s = (s.astype(dt).astype(jnp.float32) * scale).astype(dt).astype(jnp.float32)
        s = jnp.where((rel >= 0) & (rel < _W), s, mask_value)
        e = jnp.exp(s - jnp.max(s, axis=1, keepdims=True))
        p = e / jnp.sum(e, axis=1, keepdims=True)
        o = jnp.dot(p.astype(dt), v_ref[...], preferred_element_type=jnp.float32)
        o_ref[pl.ds(q0, n), :] = o.astype(o_ref.dtype)

    lax.fori_loop(0, S // n, body, None)


@jax.jit
def pallas_standalone__sliding_local_fixed_window__prompt_kernel(
    q: jax.Array,
    k: jax.Array,
    v: jax.Array,
):
    B, H, S, D = q.shape
    NH = B * H
    scale = float(np.asarray(D ** -0.5, q.dtype))
    groups = NH // _WR_REGIONS
    pairs = NH // 2
    switch = NH - 2 * _NBUF
    rounds = S // _CH
    early = (groups - 1) * rounds
    assert NH % _WR_REGIONS == 0 and groups > 1 and early % (2 * _NBUF) == 0
    assert 2 * _NBUF <= _WR_REGIONS
    assert S % (2 * _CH) == 0 and _TAIL % _CH == 0 and _TAIL <= S // 2

    def head_of(pair, member):
        n = _WR_REGIONS // 2
        return member * pairs + (pair % n) * groups + pair // n

    def kernel(q_hbm, k_hbm, v_hbm, o_hbm, in_buf, out_buf, in_sem, tail_sem, out_sem):
        def start_reads(pair, half, tail=0):
            slot = pair % _NBUF
            for off in range(0, S // 2, _CH):
                row = half * (S // 2) + off
                sem = tail_sem.at[0] if off >= S // 2 - tail else in_sem.at[slot]
                for j, src in enumerate((q_hbm, k_hbm, v_hbm)):
                    for member in range(2):
                        start = head_of(pair, member) * S + row
                        pltpu.make_async_copy(
                            src.at[pl.ds(pl.multiple_of(start, _CH), _CH)],
                            in_buf.at[slot, member, j, pl.ds(pl.multiple_of(row, _CH), _CH)],
                            sem,
                        ).start(priority=member)

        def wait_fill(buf, sem):
            pltpu.make_async_copy(buf, buf, sem).wait()

        def start_writes(lo, hi):
            def one_round(x, _):
                for r in range(_WR_REGIONS):
                    rows = pl.ds(pl.multiple_of(r * groups * S + x * _CH, _CH), _CH)
                    pltpu.make_async_copy(
                        out_buf.at[rows], o_hbm.at[rows], out_sem.at[0]
                    ).start(priority=r % 2)

            lax.fori_loop(lo, hi, one_round, None)

        last_slot = (pairs - 1) % _NBUF

        def step(i, _):
            pair, member = i // 2, i % 2
            slot = pair % _NBUF

            @pl.when(i < switch)
            def _():
                start_reads(pair + _NBUF - 1, member)

                @pl.when(member == 0)
                def _():
                    wait_fill(in_buf.at[slot], in_sem.at[slot])

            @pl.when(i == switch)
            def _():
                start_reads(pairs - 1, 0)
                start_reads(pairs - 1, 1, tail=_TAIL)
                for t in range(pairs - _NBUF, pairs - 1):
                    wait_fill(in_buf.at[t % _NBUF], in_sem.at[t % _NBUF])
                wait_fill(in_buf.at[last_slot, :, :, pl.ds(0, S - _TAIL)],
                          in_sem.at[last_slot])

            @pl.when(i >= switch)
            def _():
                per_step = early // (2 * _NBUF)
                start_writes((i - switch) * per_step, (i - switch + 1) * per_step)

            @pl.when(i == NH - 2)
            def _():
                wait_fill(in_buf.at[last_slot, :, :, pl.ds(S - _TAIL, _TAIL)],
                          tail_sem.at[0])

            rows = pl.ds(pl.multiple_of(head_of(pair, member) * S, S), S)
            refs = [in_buf.at[slot, member, j] for j in range(3)] + [out_buf.at[rows]]
            m_min = _banded_head(*refs, scale)

            @pl.when(jnp.logical_not(m_min * scale > 0.9 * _MASK_VALUE))
            def _():
                _dense_head(*refs, scale)

        lax.fori_loop(0, 2 * (_NBUF - 1), lambda i, _: start_reads(i // 2, i % 2), None)
        lax.fori_loop(0, NH, step, None)
        start_writes(early, groups * rounds)
        pltpu.make_async_copy(out_buf, o_hbm, out_sem.at[0]).wait()

    hbm = pl.BlockSpec(memory_space=pl.ANY)
    o = pl.pallas_call(
        kernel,
        in_specs=[hbm, hbm, hbm],
        out_specs=hbm,
        out_shape=jax.ShapeDtypeStruct((NH * S, D), q.dtype),
        scratch_shapes=[
            pltpu.VMEM((_NBUF, 2, 3, S, D), q.dtype),
            pltpu.VMEM((NH * S, D), q.dtype),
            pltpu.SemaphoreType.DMA((_NBUF,)),
            pltpu.SemaphoreType.DMA((1,)),
            pltpu.SemaphoreType.DMA((1,)),
        ],
        compiler_params=pltpu.CompilerParams(vmem_limit_bytes=64 * 1024 * 1024),
    )(q.reshape(NH * S, D), k.reshape(NH * S, D), v.reshape(NH * S, D))
    return o.reshape(B, H, S, D)
```
